```python
import jax
import jax.numpy as jnp

def _softmax(x, axis=-1):
    return jax.nn.softmax(x, axis=axis)
def _gelu(x):
    return jax.nn.gelu(x, approximate=True)
def _silu(x):
    return jax.nn.silu(x)
def _sigmoid(x):
    return jax.nn.sigmoid(x)
def _layernorm(x, axis=-1, eps=1e-5):
    m = jnp.mean(x, axis=axis, keepdims=True)
    v = jnp.var(x, axis=axis, keepdims=True)
    return (x - m) / jnp.sqrt(v + eps)
def _scatter_add(tgt, idx, src, axis=0):
    return tgt.at[idx].add(src)
def _segment_sum(src, seg, n):
    return jax.ops.segment_sum(src, seg, n)
class _Rng:
    def __init__(self, key):
        self._k = key
    def _next(self):
        self._k, sub = jax.random.split(self._k)
        return sub
    def normal(self, shape):
        return jax.random.normal(self._next(), shape, dtype=jnp.bfloat16)
    def randint(self, lo, hi, shape):
        return jax.random.randint(self._next(), shape, lo, hi, dtype=jnp.int32)
    def uniform(self, shape, lo=0.0, hi=1.0):
        return jax.random.uniform(self._next(), shape, jnp.bfloat16, lo, hi)
    def permutation(self, n):
        return jax.random.permutation(self._next(), n)


kernel_name = 'standalone__qk_norm__prompt'

def setup_inputs():
    _rng = _Rng(jax.random.key(int.from_bytes(__import__("os").urandom(4), "little")))
    _w = (lambda a: (lambda t: t.astype(jnp.bfloat16) if jnp.issubdtype(t.dtype, jnp.floating) else t)(jnp.asarray(a)))
    B, H, S, D = 2, 32, 2048, 1024
    Dh = D // H
    return {
        "q": _w((lambda *s: _rng.normal(s) * 0.05)(B, H, S, Dh)),
        "k": _w((lambda *s: _rng.normal(s) * 0.05)(B, H, S, Dh)),
        "v": _w((lambda *s: _rng.normal(s) * 0.05)(B, H, S, Dh)),
        "t": _w(jnp.abs((lambda *s: _rng.normal(s) * 0.05)(H)) + 1.0),
    }

def reference(q, k, v, t):
    eps = 1e-6
    qn = q / (jnp.sqrt((q * q).sum(axis=-1, keepdims=True)) + eps)
    kn = k / (jnp.sqrt((k * k).sum(axis=-1, keepdims=True)) + eps)
    logits = jnp.einsum('bhqd,bhkd->bhqk', qn, kn) * t[None, :, None, None]
    attn = _softmax(logits, axis=-1)
    return jnp.einsum('bhqk,bhkd->bhqd', attn, v)
```

```python
import jax
import jax.numpy as jnp
from jax import lax
import jax.experimental.pallas as pl
import jax.experimental.pallas.tpu as pltpu

_LOG2E = 1.4426950408889634
_EPS = 1e-6
_T_SAFE = 8.0
_F32 = jnp.float32
_BF16 = jnp.bfloat16

_BQ = 512
_BK = 512
_PC = 512
_SQ = 128


def _unit(x):
    x = x.astype(_F32)
    return x / (jnp.sqrt(jnp.sum(x * x, axis=0, keepdims=True)) + _EPS)


def _kernel(t_ref, qn_ref, kn_ref, v_ref, q0_ref, k0_ref, o_ref,
            ks_ref, qs_ref, safe_ref):
    S = v_ref.shape[-1]
    H = t_ref.shape[0]
    g = pl.program_id(0)
    h = lax.rem(g, H)
    hn = lax.rem(jnp.minimum(g + 1, pl.num_programs(0) - 1), H)
    cur = lax.rem(g, 2)
    nxt = 1 - cur
    npre = S // _PC

    def prep(qsrc, ksrc, slot, scale, i):
        sl = slice(i * _PC, (i + 1) * _PC)
        qs_ref[slot, :, sl] = (_unit(qsrc[:, sl]) * scale).astype(_BF16)
        ks_ref[slot, sl, :] = _unit(ksrc[:, sl]).T.astype(_BF16)

    @pl.when(g == 0)
    def _first():
        ok = jnp.int32(1)
        for i in range(H):
            ok = ok & (jnp.abs(t_ref[i]) <= _T_SAFE).astype(jnp.int32)
        safe_ref[0] = ok
        scale0 = jnp.where(ok == 1, t_ref[0] * _LOG2E, 1.0)
        for i in range(npre):
            prep(q0_ref, k0_ref, 0, scale0, i)

    safe = safe_ref[0] == 1

    @pl.when(safe)
    def _fast():
        cn = t_ref[hn] * _LOG2E
        nq, nk = S // _BQ, S // _BK
        steps = [(qi, ki) for qi in range(nq) for ki in range(nk)]

        def sdot(n):
            qi, ki = steps[n]
            return jnp.dot(ks_ref[cur, ki * _BK:(ki + 1) * _BK, :],
                           qs_ref[cur, :, qi * _BQ:(qi + 1) * _BQ],
                           preferred_element_type=_F32)

        every = len(steps) // (npre + 1)
        s_next = sdot(0)
        acc = l = None
        for n, (qi, ki) in enumerate(steps):
            s = s_next
            if n + 1 < len(steps):
                s_next = sdot(n + 1)
            if n % every == 0 and 1 <= n // every <= npre:
                prep(qn_ref, kn_ref, nxt, cn, n // every - 1)
            p = jnp.exp2(s)
            ls = jnp.sum(p.reshape(_BK // 8, 8, _BQ), axis=0)
            l = ls if ki == 0 else l + ls
            pv = jnp.dot(v_ref[:, ki * _BK:(ki + 1) * _BK], p.astype(_BF16),
                         preferred_element_type=_F32)
            acc = pv if ki == 0 else acc + pv
            if ki == nk - 1:
                lsum = jnp.sum(l, axis=0, keepdims=True)
                o_ref[:, qi * _BQ:(qi + 1) * _BQ] = (acc / lsum).astype(o_ref.dtype)

    @pl.when(jnp.logical_not(safe))
    def _fallback():
        for i in range(npre):
            prep(qn_ref, kn_ref, nxt, 1.0, i)
        th = t_ref[h]

        def body(i, carry):
            col = pl.ds(pl.multiple_of(i * _SQ, _SQ), _SQ)
            s = jnp.dot(ks_ref[cur], qs_ref[cur, :, col],
                        preferred_element_type=_F32) * th
            m = jnp.max(s, axis=0, keepdims=True)
            p = jnp.exp(s - m)
            w = p / jnp.sum(p, axis=0, keepdims=True)
            o = jnp.dot(v_ref[...], w.astype(_BF16), preferred_element_type=_F32)
            o_ref[:, col] = o.astype(o_ref.dtype)
            return carry

        lax.fori_loop(0, S // _SQ, body, 0)


@jax.jit
def pallas_standalone__qk_norm__prompt_kernel(
    q: jax.Array,
    k: jax.Array,
    v: jax.Array,
    t: jax.Array,
):
    B, H, S, D = q.shape
    N = B * H
    qt, kt, vt = (jnp.swapaxes(x, 2, 3).reshape(N, D, S) for x in (q, k, v))
    cur = pl.BlockSpec((None, D, S), lambda g: (g, 0, 0))
    nxt = pl.BlockSpec((None, D, S), lambda g: (jnp.minimum(g + 1, N - 1), 0, 0))
    first = pl.BlockSpec((None, D, S), lambda g: (0, 0, 0))
    o = pl.pallas_call(
        _kernel,
        grid=(N,),
        in_specs=[pl.BlockSpec(memory_space=pltpu.SMEM), nxt, nxt, cur, first, first],
        out_specs=cur,
        out_shape=jax.ShapeDtypeStruct((N, D, S), q.dtype),
        scratch_shapes=[
            pltpu.VMEM((2, S, D), _BF16),
            pltpu.VMEM((2, D, S), _BF16),
            pltpu.SMEM((1,), jnp.int32),
        ],
        compiler_params=pltpu.CompilerParams(dimension_semantics=("arbitrary",)),
        name="qk_norm_attention",
    )(t.astype(_F32), qt, kt, vt, qt, kt)
    return jnp.swapaxes(o.reshape(B, H, D, S), 2, 3)
```

```python
import jax
import jax.numpy as jnp
from jax import lax
import jax.experimental.pallas as pl
import jax.experimental.pallas.tpu as pltpu

_LOG2E = 1.4426950408889634
_EPS = 1e-6
_T_SAFE = 8.0
_F32 = jnp.float32
_BF16 = jnp.bfloat16

_BQ = 256
_BK = 512
_LA = 2
_PC = 512
_SQ = 128


def _unit(x):
    x = x.astype(_F32)
    return x / (jnp.sqrt(jnp.sum(x * x, axis=0, keepdims=True)) + _EPS)


def _kernel(t_ref, q_hbm, k_hbm, v_hbm, o_hbm,
            qb, kb, vb, ob, ks_ref, qs_ref, sem):
    N, D, S = q_hbm.shape
    H = t_ref.shape[0]
    npre = S // _PC

    def cp_q(n, slot):
        return pltpu.make_async_copy(q_hbm.at[n], qb.at[slot], sem.at[0, slot])

    def cp_k(n, slot):
        return pltpu.make_async_copy(k_hbm.at[n], kb.at[slot], sem.at[1, slot])

    def cp_v(n, slot):
        return pltpu.make_async_copy(v_hbm.at[n], vb.at[slot], sem.at[2, slot])

    def cp_o(n, slot):
        return pltpu.make_async_copy(ob.at[slot], o_hbm.at[n], sem.at[3, slot])

    def prep(slot, scale, i):
        sl = slice(i * _PC, (i + 1) * _PC)
        qs_ref[slot, :, sl] = (_unit(qb[slot, :, sl]) * scale).astype(_BF16)
        ks_ref[slot, sl, :] = _unit(kb[slot, :, sl]).T.astype(_BF16)

    for cp in (cp_q, cp_k):
        cp(0, 0).start()
    cp_v(0, 0).start()
    for cp in (cp_q, cp_k):
        cp(min(1, N - 1), 1).start()
    ob[1] = jnp.zeros(ob.shape[1:], ob.dtype)

    safe = jnp.abs(t_ref[0]) <= _T_SAFE
    for i in range(1, H):
        safe = jnp.logical_and(safe, jnp.abs(t_ref[i]) <= _T_SAFE)

    cp_q(0, 0).wait()
    cp_k(0, 0).wait()
    scale0 = jnp.where(safe, t_ref[0] * _LOG2E, 1.0)
    for i in range(npre):
        prep(0, scale0, i)
    cp_q(0, 1).wait()
    cp_k(0, 1).wait()
    cp_v(0, 0).wait()

    def head_loop(attend):
        def body(n, carry):
            cur = n & 1
            nxt = 1 - cur
            n1 = jnp.minimum(n + 1, N - 1)
            n2 = jnp.minimum(n + 2, N - 1)
            nprev = jnp.maximum(n - 1, 0)
            cp_q(n2, cur).start()
            cp_k(n2, cur).start()
            cp_v(n1, nxt).start()
            cp_o(nprev, nxt).start()
            attend(n, n1, cur, nxt)
            cp_o(nprev, nxt).wait()
            cp_q(n2, cur).wait()
            cp_k(n2, cur).wait()
            cp_v(n1, nxt).wait()
            return carry
        lax.fori_loop(0, N, body, 0)

    def head_of(n):
        return n & (H - 1) if H & (H - 1) == 0 else lax.rem(n, H)

    def attend_bounded(n, n1, cur, nxt):
        scale_next = t_ref[head_of(n1)] * _LOG2E
        nq, nk = S // _BQ, S // _BK
        steps = [(qi, ki) for qi in range(nq) for ki in range(nk)]
        every = len(steps) // npre

        def sdot(m):
            qi, ki = steps[m]
            return jnp.dot(ks_ref[cur, ki * _BK:(ki + 1) * _BK, :],
                           qs_ref[cur, :, qi * _BQ:(qi + 1) * _BQ],
                           preferred_element_type=_F32)

        pend = [sdot(m) for m in range(_LA)]
        acc = l = None
        for m, (qi, ki) in enumerate(steps):
            if m + _LA < len(steps):
                pend.append(sdot(m + _LA))
            if m % every == 0:
                prep(nxt, scale_next, m // every)
            p = jnp.exp2(pend.pop(0))
            ls = jnp.sum(p.reshape(_BK // 8, 8, _BQ), axis=0)
            l = ls if ki == 0 else l + ls
            pv = jnp.dot(vb[cur, :, ki * _BK:(ki + 1) * _BK], p.astype(_BF16),
                         preferred_element_type=_F32)
            acc = pv if ki == 0 else acc + pv
            if ki == nk - 1:
                lsum = jnp.sum(l, axis=0, keepdims=True)
                ob[cur, :, qi * _BQ:(qi + 1) * _BQ] = (acc / lsum).astype(ob.dtype)

    def attend_general(n, n1, cur, nxt):
        for i in range(npre):
            prep(nxt, 1.0, i)
        th = t_ref[head_of(n)]

        def qblock(i, carry):
            col = pl.ds(pl.multiple_of(i * _SQ, _SQ), _SQ)
            s = jnp.dot(ks_ref[cur], qs_ref[cur, :, col],
                        preferred_element_type=_F32) * th
            p = jnp.exp(s - jnp.max(s, axis=0, keepdims=True))
            w = p / jnp.sum(p, axis=0, keepdims=True)
            o = jnp.dot(vb[cur], w.astype(_BF16), preferred_element_type=_F32)
            ob[cur, :, col] = o.astype(ob.dtype)
            return carry

        lax.fori_loop(0, S // _SQ, qblock, 0)

    @pl.when(safe)
    def _():
        head_loop(attend_bounded)

    @pl.when(jnp.logical_not(safe))
    def _():
        head_loop(attend_general)

    last = cp_o(N - 1, (N - 1) % 2)
    last.start()
    last.wait()


@jax.jit
def pallas_standalone__qk_norm__prompt_kernel(
    q: jax.Array,
    k: jax.Array,
    v: jax.Array,
    t: jax.Array,
):
    B, H, S, D = q.shape
    N = B * H
    qt, kt, vt = (jnp.swapaxes(x, 2, 3).reshape(N, D, S) for x in (q, k, v))
    hbm = pl.BlockSpec(memory_space=pl.ANY)
    head = pltpu.VMEM((2, D, S), q.dtype)
    o = pl.pallas_call(
        _kernel,
        in_specs=[pl.BlockSpec(memory_space=pltpu.SMEM), hbm, hbm, hbm],
        out_specs=hbm,
        out_shape=jax.ShapeDtypeStruct((N, D, S), q.dtype),
        scratch_shapes=[
            head, head, head, head,
            pltpu.VMEM((2, S, D), _BF16),
            pltpu.VMEM((2, D, S), _BF16),
            pltpu.SemaphoreType.DMA((4, 2)),
        ],
        name="qk_norm_attention",
    )(t.astype(_F32), qt, kt, vt)
    return jnp.swapaxes(o.reshape(B, H, D, S), 2, 3)
```

```python
import jax
import jax.numpy as jnp
from jax import lax
import jax.experimental.pallas as pl
import jax.experimental.pallas.tpu as pltpu

_LOG2E = 1.4426950408889634
_EPS = 1e-6
_T_SAFE = 8.0
_F32 = jnp.float32
_BF16 = jnp.bfloat16

_BQ = 256
_BK = 512
_LA = 2
_PC = 512
_SQ = 128


def _unit(x):
    x = x.astype(_F32)
    return x / (jnp.sqrt(jnp.sum(x * x, axis=0, keepdims=True)) + _EPS)


def _kernel(t_ref, q_hbm, k_hbm, v_hbm, o_hbm,
            qb, kb, vb, ob, ks_ref, qs_ref, sem):
    N, D, S = q_hbm.shape
    H = t_ref.shape[0]
    npre = S // _PC

    def cp_q(n, slot):
        return pltpu.make_async_copy(q_hbm.at[n], qb.at[slot], sem.at[0, slot])

    def cp_k(n, slot):
        return pltpu.make_async_copy(k_hbm.at[n], kb.at[slot], sem.at[1, slot])

    def cp_v(n, slot):
        return pltpu.make_async_copy(v_hbm.at[n], vb.at[slot], sem.at[2, slot])

    def cp_o(n, slot):
        return pltpu.make_async_copy(ob.at[slot], o_hbm.at[n], sem.at[3, slot])

    def prep(slot, scale, i):
        sl = slice(i * _PC, (i + 1) * _PC)
        qs_ref[slot, :, sl] = (_unit(qb[slot, :, sl]) * scale).astype(_BF16)
        ks_ref[slot, sl, :] = _unit(kb[slot, :, sl]).T.astype(_BF16)

    for cp in (cp_q, cp_k):
        cp(0, 0).start()
    cp_v(0, 0).start()
    for cp in (cp_q, cp_k):
        cp(min(1, N - 1), 1).start()
    ob[1] = jnp.zeros(ob.shape[1:], ob.dtype)

    def temp(i):
        return t_ref[i].astype(_F32)

    safe = jnp.abs(temp(0)) <= _T_SAFE
    for i in range(1, H):
        safe = jnp.logical_and(safe, jnp.abs(temp(i)) <= _T_SAFE)

    cp_q(0, 0).wait()
    cp_k(0, 0).wait()
    scale0 = jnp.where(safe, temp(0) * _LOG2E, 1.0)
    for i in range(npre):
        prep(0, scale0, i)
    cp_q(0, 1).wait()
    cp_k(0, 1).wait()
    cp_v(0, 0).wait()

    def head_loop(attend):
        def body(n, carry):
            cur = n & 1
            nxt = 1 - cur
            n1 = jnp.minimum(n + 1, N - 1)
            n2 = jnp.minimum(n + 2, N - 1)
            nprev = jnp.maximum(n - 1, 0)
            cp_q(n2, cur).start()
            cp_k(n2, cur).start()
            cp_v(n1, nxt).start()
            cp_o(nprev, nxt).start()
            attend(n, n1, cur, nxt)
            cp_o(nprev, nxt).wait()
            cp_q(n2, cur).wait()
            cp_k(n2, cur).wait()
            cp_v(n1, nxt).wait()
            return carry
        lax.fori_loop(0, N, body, 0)

    def head_of(n):
        return n & (H - 1) if H & (H - 1) == 0 else lax.rem(n, H)

    def attend_bounded(n, n1, cur, nxt):
        scale_next = temp(head_of(n1)) * _LOG2E
        nq, nk = S // _BQ, S // _BK
        steps = [(qi, ki) for qi in range(nq) for ki in range(nk)]
        every = len(steps) // npre

        def sdot(m):
            qi, ki = steps[m]
            return jnp.dot(ks_ref[cur, ki * _BK:(ki + 1) * _BK, :],
                           qs_ref[cur, :, qi * _BQ:(qi + 1) * _BQ],
                           preferred_element_type=_F32)

        pend = [sdot(m) for m in range(_LA)]
        acc = l = None
        for m, (qi, ki) in enumerate(steps):
            if m + _LA < len(steps):
                pend.append(sdot(m + _LA))
            if m % every == 0:
                prep(nxt, scale_next, m // every)
            p = jnp.exp2(pend.pop(0))
            ls = jnp.sum(p.reshape(_BK // 8, 8, _BQ), axis=0)
            l = ls if ki == 0 else l + ls
            pv = jnp.dot(vb[cur, :, ki * _BK:(ki + 1) * _BK], p.astype(_BF16),
                         preferred_element_type=_F32)
            acc = pv if ki == 0 else acc + pv
            if ki == nk - 1:
                lsum = jnp.sum(l, axis=0, keepdims=True)
                ob[cur, :, qi * _BQ:(qi + 1) * _BQ] = (acc / lsum).astype(ob.dtype)

    def attend_general(n, n1, cur, nxt):
        for i in range(npre):
            prep(nxt, 1.0, i)
        th = temp(head_of(n))

        def qblock(i, carry):
            col = pl.ds(pl.multiple_of(i * _SQ, _SQ), _SQ)
            s = jnp.dot(ks_ref[cur], qs_ref[cur, :, col],
                        preferred_element_type=_F32) * th
            p = jnp.exp(s - jnp.max(s, axis=0, keepdims=True))
            w = p / jnp.sum(p, axis=0, keepdims=True)
            o = jnp.dot(vb[cur], w.astype(_BF16), preferred_element_type=_F32)
            ob[cur, :, col] = o.astype(ob.dtype)
            return carry

        lax.fori_loop(0, S // _SQ, qblock, 0)

    @pl.when(safe)
    def _():
        head_loop(attend_bounded)

    @pl.when(jnp.logical_not(safe))
    def _():
        head_loop(attend_general)

    last = cp_o(N - 1, (N - 1) % 2)
    last.start()
    last.wait()


@jax.jit
def pallas_standalone__qk_norm__prompt_kernel(
    q: jax.Array,
    k: jax.Array,
    v: jax.Array,
    t: jax.Array,
):
    B, H, S, D = q.shape
    N = B * H
    qt, kt, vt = (jnp.swapaxes(x, 2, 3).reshape(N, D, S) for x in (q, k, v))
    hbm = pl.BlockSpec(memory_space=pl.ANY)
    head = pltpu.VMEM((2, D, S), q.dtype)
    o = pl.pallas_call(
        _kernel,
        in_specs=[pl.BlockSpec(memory_space=pltpu.SMEM), hbm, hbm, hbm],
        out_specs=hbm,
        out_shape=jax.ShapeDtypeStruct((N, D, S), q.dtype),
        scratch_shapes=[
            head, head, head, head,
            pltpu.VMEM((2, S, D), _BF16),
            pltpu.VMEM((2, D, S), _BF16),
            pltpu.SemaphoreType.DMA((4, 2)),
        ],
        name="qk_norm_attention",
    )(t, qt, kt, vt)
    return jnp.swapaxes(o.reshape(B, H, D, S), 2, 3)
```

```python
import jax
import jax.numpy as jnp
from jax import lax
import jax.experimental.pallas as pl
import jax.experimental.pallas.tpu as pltpu

_LOG2E = 1.4426950408889634
_EPS = 1e-6
_T_SAFE = 8.0
_F32 = jnp.float32
_BF16 = jnp.bfloat16

_HB = 4
_PC = 512
_SQ = 128
_CFG_ONE = (256, 512, 2, 0, 8)
_CFG_MAIN = (512, 512, 1, 2, 2)


def _unit(x):
    x = x.astype(_F32)
    return x / (jnp.sqrt(jnp.sum(x * x, axis=0, keepdims=True)) + _EPS)


def _kernel(t_ref, q_hbm, k_hbm, v_hbm, o_hbm,
            qa, ka, va, oa, qb, kb, vb, ob, ks_ref, qs_ref, temp_ref,
            sem_a, sem_b, sem_o):
    N, D, S = q_hbm.shape
    H = t_ref.shape[0]
    hb = _HB
    npre = S // _PC
    n_one = (N % hb or hb) if N >= 2 * hb else N
    n_blk = (N - n_one) // hb
    copy = pltpu.make_async_copy
    every = slice(None)

    def temp(n):
        return temp_ref[n & (H - 1) if H & (H - 1) == 0 else lax.rem(n, H)]

    def prep(qsrc, ksrc, idx, slot, scale, i):
        sl = slice(i * _PC, (i + 1) * _PC)
        qs_ref[slot, :, sl] = (_unit(qsrc[idx + (every, sl)]) * scale).astype(_BF16)
        ks_ref[slot, sl, :] = _unit(ksrc[idx + (every, sl)]).T.astype(_BF16)

    def attend_bounded(cfg, nheads, slot, vsrc, odst, idx, prep_next, after_head):
        bq, bk, la, pstart, pevery = cfg
        nq, nk = S // bq, S // bk
        steps = [(j, qi, ki) for j in range(nheads)
                 for qi in range(nq) for ki in range(nk)]

        def sdot(m):
            j, qi, ki = steps[m]
            return jnp.dot(ks_ref[slot(j), ki * bk:(ki + 1) * bk, :],
                           qs_ref[slot(j), :, qi * bq:(qi + 1) * bq],
                           preferred_element_type=_F32)

        pend = [sdot(m) for m in range(la)]
        acc = l = None
        for m, (j, qi, ki) in enumerate(steps):
            r = m % (nq * nk)
            if m + la < len(steps):
                pend.append(sdot(m + la))
            if r % pevery == 0 and pstart <= r // pevery < pstart + npre:
                prep_next(j, r // pevery - pstart)
            p = jnp.exp2(pend.pop(0))
            ls = jnp.sum(p.reshape(bk // 8, 8, bq), axis=0)
            l = ls if ki == 0 else l + ls
            vt = vsrc[idx(j) + (every, slice(ki * bk, (ki + 1) * bk))]
            pv = jnp.dot(vt, p.astype(_BF16), preferred_element_type=_F32)
            acc = pv if ki == 0 else acc + pv
            if ki == nk - 1:
                lsum = jnp.sum(l, axis=0, keepdims=True)
                odst[idx(j) + (every, slice(qi * bq, (qi + 1) * bq))] = (
                    acc / lsum).astype(odst.dtype)
                if qi == nq - 1:
                    after_head(j)

    def attend_general(n, cur):
        th = temp(n)

        def qblock(i, carry):
            col = pl.ds(pl.multiple_of(i * _SQ, _SQ), _SQ)
            s = jnp.dot(ks_ref[cur], qs_ref[cur, :, col],
                        preferred_element_type=_F32) * th
            p = jnp.exp(s - jnp.max(s, axis=0, keepdims=True))
            w = p / jnp.sum(p, axis=0, keepdims=True)
            o = jnp.dot(va[cur], w.astype(_BF16), preferred_element_type=_F32)
            oa[cur, :, col] = o.astype(oa.dtype)
            return carry

        lax.fori_loop(0, S // _SQ, qblock, 0)

    def a_q(n, s):
        return copy(q_hbm.at[n], qa.at[s], sem_a.at[0, s])

    def a_k(n, s):
        return copy(k_hbm.at[n], ka.at[s], sem_a.at[1, s])

    def a_v(n, s):
        return copy(v_hbm.at[n], va.at[s], sem_a.at[2, s])

    def a_o(n, s):
        return copy(oa.at[s], o_hbm.at[n], sem_a.at[3, s])

    def run_one_by_one(count, attend):
        top = min(count, N - 1)

        def body(n, carry):
            cur = n & 1
            nxt = 1 - cur
            n1 = jnp.minimum(n + 1, N - 1)
            n2 = jnp.minimum(n + 2, top)
            nv = jnp.minimum(n + 1, count - 1)
            nprev = jnp.maximum(n - 1, 0)
            loads = [a_q(n2, cur), a_k(n2, cur), a_v(nv, nxt)]
            store = a_o(nprev, nxt)
            for c in loads:
                c.start()
            store.start()
            attend(n, n1, cur, nxt)
            store.wait()
            for c in loads:
                c.wait()
            return carry

        lax.fori_loop(0, count, body, 0)
        last = a_o(count - 1, (count - 1) % 2)
        last.start()
        return last

    def b_loads(i, s):
        h0 = n_one + i * hb
        hl = jnp.minimum(h0 + hb, N - 1)
        return [
            copy(q_hbm.at[pl.ds(h0 + 1, hb - 1)], qb.at[s, pl.ds(0, hb - 1)], sem_b.at[0, s]),
            copy(q_hbm.at[hl], qb.at[s, hb - 1], sem_b.at[1, s]),
            copy(k_hbm.at[pl.ds(h0 + 1, hb - 1)], kb.at[s, pl.ds(0, hb - 1)], sem_b.at[2, s]),
            copy(k_hbm.at[hl], kb.at[s, hb - 1], sem_b.at[3, s]),
            copy(v_hbm.at[pl.ds(h0, hb)], vb.at[s], sem_b.at[4, s]),
        ]

    def b_o(i, s, j):
        return copy(ob.at[s, j], o_hbm.at[n_one + i * hb + j], sem_o.at[s, j])

    def run_blocks(zero):
        def body(it, carry):
            cur = it & 1
            nxt = 1 - cur
            loads = b_loads(jnp.minimum(it + 1, n_blk - 1), nxt)
            late_store = b_o(jnp.maximum(it - 1, 0), nxt, hb - 1)
            for c in loads:
                c.start()
            late_store.start()

            def slot(j):
                return ((n_one + j) & 1) + zero

            def prep_next(j, i):
                n1 = jnp.minimum(n_one + it * hb + j + 1, N - 1)
                prep(qb, kb, (cur, j), slot(j + 1), temp(n1) * _LOG2E, i)

            def after_head(j):
                if j < hb - 1:
                    b_o(it, cur, j).start()

            attend_bounded(_CFG_MAIN, hb, slot, vb, ob, lambda j: (cur, j),
                           prep_next, after_head)
            late_store.wait()
            for j in range(hb - 1):
                b_o(it, cur, j).wait()
            for c in loads:
                c.wait()
            return carry

        lax.fori_loop(0, n_blk, body, 0)
        last = b_o(n_blk - 1, (n_blk - 1) % 2, hb - 1)
        last.start()
        return last

    first = [a_q(0, 0), a_k(0, 0)]
    second = [a_v(0, 0), a_q(min(1, N - 1), 1), a_k(min(1, N - 1), 1)]
    for c in first + second:
        c.start()
    oa[1] = jnp.zeros(oa.shape[1:], oa.dtype)
    safe = None
    for i in range(H):
        ti = t_ref[i].astype(_F32)
        temp_ref[i] = ti
        ok = jnp.abs(ti) <= _T_SAFE
        safe = ok if safe is None else jnp.logical_and(safe, ok)
    for c in first:
        c.wait()
    scale0 = jnp.where(safe, temp_ref[0] * _LOG2E, 1.0)
    for i in range(npre):
        prep(qa, ka, (0,), 0, scale0, i)
    for c in second:
        c.wait()

    @pl.when(safe)
    def _bounded():
        if n_blk:
            for c in b_loads(0, 0):
                c.start()
            ob[1, hb - 1] = jnp.zeros(ob.shape[2:], ob.dtype)

        def attend(n, n1, cur, nxt):
            scale = temp(n1) * _LOG2E
            attend_bounded(_CFG_ONE, 1, lambda j: cur, va, oa, lambda j: (cur,),
                           lambda j, i: prep(qa, ka, (nxt,), nxt, scale, i),
                           lambda j: None)

        pending = [run_one_by_one(n_one, attend)]
        if n_blk:
            for c in b_loads(0, 0):
                c.wait()
            zero = (temp_ref[0] > 2 * _T_SAFE).astype(jnp.int32)
            pending.append(run_blocks(zero))
        for c in pending:
            c.wait()

    @pl.when(jnp.logical_not(safe))
    def _general():
        def attend(n, n1, cur, nxt):
            for i in range(npre):
                prep(qa, ka, (nxt,), nxt, 1.0, i)
            attend_general(n, cur)

        run_one_by_one(N, attend).wait()


@jax.jit
def pallas_standalone__qk_norm__prompt_kernel(
    q: jax.Array,
    k: jax.Array,
    v: jax.Array,
    t: jax.Array,
):
    B, H, S, D = q.shape
    N = B * H
    qt, kt, vt = (jnp.swapaxes(x, 2, 3).reshape(N, D, S) for x in (q, k, v))
    hbm = pl.BlockSpec(memory_space=pl.ANY)
    one = pltpu.VMEM((2, D, S), q.dtype)
    blk = pltpu.VMEM((2, _HB, D, S), q.dtype)
    o = pl.pallas_call(
        _kernel,
        in_specs=[pl.BlockSpec(memory_space=pltpu.SMEM), hbm, hbm, hbm],
        out_specs=hbm,
        out_shape=jax.ShapeDtypeStruct((N, D, S), q.dtype),
        scratch_shapes=[
            one, one, one, one,
            blk, blk, blk, blk,
            pltpu.VMEM((3, S, D), _BF16),
            pltpu.VMEM((3, D, S), _BF16),
            pltpu.SMEM((H,), _F32),
            pltpu.SemaphoreType.DMA((4, 2)),
            pltpu.SemaphoreType.DMA((5, 2)),
            pltpu.SemaphoreType.DMA((2, _HB)),
        ],
        compiler_params=pltpu.CompilerParams(vmem_limit_bytes=48 * 1024 * 1024),
        name="qk_norm_attention",
    )(t, qt, kt, vt)
    return jnp.swapaxes(o.reshape(B, H, D, S), 2, 3)
```

```python
import jax
import jax.numpy as jnp
from jax import lax
import jax.experimental.pallas as pl
import jax.experimental.pallas.tpu as pltpu

_LOG2E = 1.4426950408889634
_EPS = 1e-6
_T_SAFE = 8.0
_F32 = jnp.float32
_BF16 = jnp.bfloat16

_HB = 4
_PC = 512
_SQ = 128
_CFG_ONE = (256, 512, 2, 0, 8)
_CFG_MAIN = (1024, 128, 1, 2, 4)


def _unit(x):
    x = x.astype(_F32)
    return x / (jnp.sqrt(jnp.sum(x * x, axis=0, keepdims=True)) + _EPS)


def _kernel(t_hbm, q_hbm, k_hbm, v_hbm, o_hbm,
            qa, ka, va, oa, qb, kb, vb, ob, ks_ref, qs_ref, t_ref, temp_ref,
            sem_a, sem_b, sem_o, sem_t):
    N, D, S = q_hbm.shape
    H = t_ref.shape[0]
    hb = _HB
    npre = S // _PC
    n_one = (N % hb or hb) if N >= 2 * hb else N
    n_blk = (N - n_one) // hb
    copy = pltpu.make_async_copy
    every = slice(None)

    def temp(n):
        return temp_ref[n & (H - 1) if H & (H - 1) == 0 else lax.rem(n, H)]

    def prep(qsrc, ksrc, idx, slot, scale, i):
        sl = slice(i * _PC, (i + 1) * _PC)
        qs_ref[slot, :, sl] = (_unit(qsrc[idx + (every, sl)]) * scale).astype(_BF16)
        ks_ref[slot, sl, :] = _unit(ksrc[idx + (every, sl)]).T.astype(_BF16)

    def attend_bounded(cfg, nheads, slot, vsrc, odst, idx, prep_next, after_head):
        bq, bk, la, pstart, pevery = cfg
        nq, nk = S // bq, S // bk
        steps = [(j, qi, ki) for j in range(nheads)
                 for qi in range(nq) for ki in range(nk)]

        def sdot(m):
            j, qi, ki = steps[m]
            return jnp.dot(ks_ref[slot(j), ki * bk:(ki + 1) * bk, :],
                           qs_ref[slot(j), :, qi * bq:(qi + 1) * bq],
                           preferred_element_type=_F32)

        pend = [sdot(m) for m in range(la)]
        acc = l = None
        for m, (j, qi, ki) in enumerate(steps):
            r = m % (nq * nk)
            if m + la < len(steps):
                pend.append(sdot(m + la))
            if r % pevery == 0 and pstart <= r // pevery < pstart + npre:
                prep_next(j, r // pevery - pstart)
            p = jnp.exp2(pend.pop(0))
            ls = jnp.sum(p.reshape(bk // 8, 8, bq), axis=0)
            l = ls if ki == 0 else l + ls
            vt = vsrc[idx(j) + (every, slice(ki * bk, (ki + 1) * bk))]
            pv = jnp.dot(vt, p.astype(_BF16), preferred_element_type=_F32)
            acc = pv if ki == 0 else acc + pv
            if ki == nk - 1:
                lsum = jnp.sum(l, axis=0, keepdims=True)
                odst[idx(j) + (every, slice(qi * bq, (qi + 1) * bq))] = (
                    acc / lsum).astype(odst.dtype)
                if qi == nq - 1:
                    after_head(j)

    def attend_general(n, cur):
        th = temp(n)

        def qblock(i, carry):
            col = pl.ds(pl.multiple_of(i * _SQ, _SQ), _SQ)
            s = jnp.dot(ks_ref[cur], qs_ref[cur, :, col],
                        preferred_element_type=_F32) * th
            p = jnp.exp(s - jnp.max(s, axis=0, keepdims=True))
            w = p / jnp.sum(p, axis=0, keepdims=True)
            o = jnp.dot(va[cur], w.astype(_BF16), preferred_element_type=_F32)
            oa[cur, :, col] = o.astype(oa.dtype)
            return carry

        lax.fori_loop(0, S // _SQ, qblock, 0)

    def a_q(n, s):
        return copy(q_hbm.at[n], qa.at[s], sem_a.at[0, s])

    def a_k(n, s):
        return copy(k_hbm.at[n], ka.at[s], sem_a.at[1, s])

    def a_v(n, s):
        return copy(v_hbm.at[n], va.at[s], sem_a.at[2, s])

    def a_o(n, s):
        return copy(oa.at[s], o_hbm.at[n], sem_a.at[3, s])

    def run_one_by_one(count, attend):
        top = min(count, N - 1)

        def body(n, carry):
            cur = n & 1
            nxt = 1 - cur
            n1 = jnp.minimum(n + 1, N - 1)
            n2 = jnp.minimum(n + 2, top)
            nv = jnp.minimum(n + 1, count - 1)
            nprev = jnp.maximum(n - 1, 0)
            loads = [a_q(n2, cur), a_k(n2, cur), a_v(nv, nxt)]
            store = a_o(nprev, nxt)
            for c in loads:
                c.start()
            store.start()
            attend(n, n1, cur, nxt)
            store.wait()
            for c in loads:
                c.wait()
            return carry

        lax.fori_loop(0, count, body, 0)
        last = a_o(count - 1, (count - 1) % 2)
        last.start()
        return last

    def b_loads(i, s):
        h0 = n_one + i * hb
        hl = jnp.minimum(h0 + hb, N - 1)
        return [
            copy(q_hbm.at[pl.ds(h0 + 1, hb - 1)], qb.at[s, pl.ds(0, hb - 1)], sem_b.at[0, s]),
            copy(q_hbm.at[hl], qb.at[s, hb - 1], sem_b.at[1, s]),
            copy(k_hbm.at[pl.ds(h0 + 1, hb - 1)], kb.at[s, pl.ds(0, hb - 1)], sem_b.at[2, s]),
            copy(k_hbm.at[hl], kb.at[s, hb - 1], sem_b.at[3, s]),
            copy(v_hbm.at[pl.ds(h0, hb)], vb.at[s], sem_b.at[4, s]),
        ]

    def b_o(i, s, j):
        return copy(ob.at[s, j], o_hbm.at[n_one + i * hb + j], sem_o.at[s, j])

    def run_blocks(zero):
        def body(it, carry):
            cur = it & 1
            nxt = 1 - cur
            loads = b_loads(jnp.minimum(it + 1, n_blk - 1), nxt)
            late_store = b_o(jnp.maximum(it - 1, 0), nxt, hb - 1)
            for c in loads:
                c.start()
            late_store.start()

            def slot(j):
                return ((n_one + j) & 1) + zero

            def prep_next(j, i):
                n1 = jnp.minimum(n_one + it * hb + j + 1, N - 1)
                prep(qb, kb, (cur, j), slot(j + 1), temp(n1) * _LOG2E, i)

            def after_head(j):
                if j < hb - 1:
                    b_o(it, cur, j).start()

            attend_bounded(_CFG_MAIN, hb, slot, vb, ob, lambda j: (cur, j),
                           prep_next, after_head)
            late_store.wait()
            for j in range(hb - 1):
                b_o(it, cur, j).wait()
            for c in loads:
                c.wait()
            return carry

        lax.fori_loop(0, n_blk, body, 0)
        last = b_o(n_blk - 1, (n_blk - 1) % 2, hb - 1)
        last.start()
        return last

    load_t = copy(t_hbm, t_ref, sem_t)
    load_t.start()
    first = [a_q(0, 0), a_k(0, 0)]
    second = [a_v(0, 0), a_q(min(1, N - 1), 1), a_k(min(1, N - 1), 1)]
    for c in first + second:
        c.start()
    oa[1] = jnp.zeros(oa.shape[1:], oa.dtype)
    load_t.wait()
    safe = None
    for i in range(H):
        ti = t_ref[i].astype(_F32)
        temp_ref[i] = ti
        ok = jnp.abs(ti) <= _T_SAFE
        safe = ok if safe is None else jnp.logical_and(safe, ok)
    for c in first:
        c.wait()
    scale0 = jnp.where(safe, temp_ref[0] * _LOG2E, 1.0)
    for i in range(npre):
        prep(qa, ka, (0,), 0, scale0, i)
    for c in second:
        c.wait()

    @pl.when(safe)
    def _bounded():
        if n_blk:
            for c in b_loads(0, 0):
                c.start()
            ob[1, hb - 1] = jnp.zeros(ob.shape[2:], ob.dtype)

        def attend(n, n1, cur, nxt):
            scale = temp(n1) * _LOG2E
            attend_bounded(_CFG_ONE, 1, lambda j: cur, va, oa, lambda j: (cur,),
                           lambda j, i: prep(qa, ka, (nxt,), nxt, scale, i),
                           lambda j: None)

        pending = [run_one_by_one(n_one, attend)]
        if n_blk:
            for c in b_loads(0, 0):
                c.wait()
            zero = (temp_ref[0] > 2 * _T_SAFE).astype(jnp.int32)
            pending.append(run_blocks(zero))
        for c in pending:
            c.wait()

    @pl.when(jnp.logical_not(safe))
    def _general():
        def attend(n, n1, cur, nxt):
            for i in range(npre):
                prep(qa, ka, (nxt,), nxt, 1.0, i)
            attend_general(n, cur)

        run_one_by_one(N, attend).wait()


@jax.jit
def pallas_standalone__qk_norm__prompt_kernel(
    q: jax.Array,
    k: jax.Array,
    v: jax.Array,
    t: jax.Array,
):
    B, H, S, D = q.shape
    N = B * H
    qt, kt, vt = (jnp.swapaxes(x, 2, 3).reshape(N, D, S) for x in (q, k, v))
    hbm = pl.BlockSpec(memory_space=pl.ANY)
    one = pltpu.VMEM((2, D, S), q.dtype)
    blk = pltpu.VMEM((2, _HB, D, S), q.dtype)
    o = pl.pallas_call(
        _kernel,
        in_specs=[hbm, hbm, hbm, hbm],
        out_specs=hbm,
        out_shape=jax.ShapeDtypeStruct((N, D, S), q.dtype),
        scratch_shapes=[
            one, one, one, one,
            blk, blk, blk, blk,
            pltpu.VMEM((3, S, D), _BF16),
            pltpu.VMEM((3, D, S), _BF16),
            pltpu.SMEM((H,), t.dtype),
            pltpu.SMEM((H,), _F32),
            pltpu.SemaphoreType.DMA((4, 2)),
            pltpu.SemaphoreType.DMA((5, 2)),
            pltpu.SemaphoreType.DMA((2, _HB)),
            pltpu.SemaphoreType.DMA,
        ],
        compiler_params=pltpu.CompilerParams(vmem_limit_bytes=48 * 1024 * 1024),
        name="qk_norm_attention",
    )(t, qt, kt, vt)
    return jnp.swapaxes(o.reshape(B, H, D, S), 2, 3)
```

```python
import jax
import jax.numpy as jnp
from jax import lax
import jax.experimental.pallas as pl
import jax.experimental.pallas.tpu as pltpu

_LOG2E = 1.4426950408889634
_EPS = 1e-6
_T_SAFE = 8.0
_F32 = jnp.float32
_BF16 = jnp.bfloat16

_HB = 4
_PC = 512
_SQ = 128
_CFG_ONE = (256, 512, 2, 0, 8)
_CFG_MAIN = (1024, 128, 1, 2, 4)


def _unit(x):
    x = x.astype(_F32)
    return x / (jnp.sqrt(jnp.sum(x * x, axis=0, keepdims=True)) + _EPS)


def _kernel(t_hbm, q_hbm, k_hbm, v_hbm, o_hbm,
            qa, ka, va, oa, qb, kb, vb, ob, ks_ref, qs_ref, t_ref, temp_ref,
            sem_a, sem_b, sem_o, sem_t):
    N, D, S = q_hbm.shape
    H = t_ref.shape[0]
    hb = _HB
    npre = S // _PC
    n_one = (N % hb or hb) if N >= 2 * hb else N
    n_blk = (N - n_one) // hb
    copy = pltpu.make_async_copy
    every = slice(None)

    def temp(n):
        return temp_ref[n & (H - 1) if H & (H - 1) == 0 else lax.rem(n, H)]

    def prep(qsrc, ksrc, idx, slot, scale, i):
        sl = slice(i * _PC, (i + 1) * _PC)
        qs_ref[slot, :, sl] = (_unit(qsrc[idx + (every, sl)]) * scale).astype(_BF16)
        ks_ref[slot, sl, :] = _unit(ksrc[idx + (every, sl)]).T.astype(_BF16)

    def attend_bounded(cfg, nheads, slot, vsrc, odst, idx, prep_next, after_head):
        bq, bk, la, pstart, pevery = cfg
        nq, nk = S // bq, S // bk
        assert S % bq == 0 and S % bk == 0
        assert nq * nk > pevery * (pstart + npre - 1)
        steps = [(j, qi, ki) for j in range(nheads)
                 for qi in range(nq) for ki in range(nk)]

        def sdot(m):
            j, qi, ki = steps[m]
            return jnp.dot(ks_ref[slot(j), ki * bk:(ki + 1) * bk, :],
                           qs_ref[slot(j), :, qi * bq:(qi + 1) * bq],
                           preferred_element_type=_F32)

        pend = [sdot(m) for m in range(la)]
        issued = la
        acc = l = None
        for m, (j, qi, ki) in enumerate(steps):
            r = m % (nq * nk)
            ahead = la if m + la + 2 < len(steps) else la + 2
            while issued < min(len(steps), m + 1 + ahead):
                pend.append(sdot(issued))
                issued += 1
            if r % pevery == 0 and pstart <= r // pevery < pstart + npre:
                prep_next(j, r // pevery - pstart)
            p = jnp.exp2(pend.pop(0))
            ls = jnp.sum(p.reshape(bk // 8, 8, bq), axis=0)
            l = ls if ki == 0 else l + ls
            vt = vsrc[idx(j) + (every, slice(ki * bk, (ki + 1) * bk))]
            pv = jnp.dot(vt, p.astype(_BF16), preferred_element_type=_F32)
            acc = pv if ki == 0 else acc + pv
            if ki == nk - 1:
                lsum = jnp.sum(l, axis=0, keepdims=True)
                odst[idx(j) + (every, slice(qi * bq, (qi + 1) * bq))] = (
                    acc / lsum).astype(odst.dtype)
                if qi == nq - 1:
                    after_head(j)

    def attend_general(n, cur):
        th = temp(n)

        def qblock(i, carry):
            col = pl.ds(pl.multiple_of(i * _SQ, _SQ), _SQ)
            s = jnp.dot(ks_ref[cur], qs_ref[cur, :, col],
                        preferred_element_type=_F32) * th
            p = jnp.exp(s - jnp.max(s, axis=0, keepdims=True))
            w = p / jnp.sum(p, axis=0, keepdims=True)
            o = jnp.dot(va[cur], w.astype(_BF16), preferred_element_type=_F32)
            oa[cur, :, col] = o.astype(oa.dtype)
            return carry

        lax.fori_loop(0, S // _SQ, qblock, 0)

    def a_q(n, s):
        return copy(q_hbm.at[n], qa.at[s], sem_a.at[0, s])

    def a_k(n, s):
        return copy(k_hbm.at[n], ka.at[s], sem_a.at[1, s])

    def a_v(n, s):
        return copy(v_hbm.at[n], va.at[s], sem_a.at[2, s])

    def a_o(n, s):
        return copy(oa.at[s], o_hbm.at[n], sem_a.at[3, s])

    def run_one_by_one(count, attend):
        top = min(count, N - 1)

        def body(n, carry):
            cur = n & 1
            nxt = 1 - cur
            n1 = jnp.minimum(n + 1, N - 1)
            n2 = jnp.minimum(n + 2, top)
            nv = jnp.minimum(n + 1, count - 1)
            nprev = jnp.maximum(n - 1, 0)
            loads = [a_q(n2, cur), a_k(n2, cur), a_v(nv, nxt)]
            store = a_o(nprev, nxt)
            for c in loads:
                c.start()
            store.start()
            attend(n, n1, cur, nxt)
            store.wait()
            for c in loads:
                c.wait()
            return carry

        lax.fori_loop(0, count, body, 0)
        last = a_o(count - 1, (count - 1) % 2)
        last.start()
        return last

    def b_loads(i, s):
        h0 = n_one + i * hb
        hl = jnp.minimum(h0 + hb, N - 1)
        return [
            copy(q_hbm.at[pl.ds(h0 + 1, hb - 1)], qb.at[s, pl.ds(0, hb - 1)], sem_b.at[0, s]),
            copy(q_hbm.at[hl], qb.at[s, hb - 1], sem_b.at[1, s]),
            copy(k_hbm.at[pl.ds(h0 + 1, hb - 1)], kb.at[s, pl.ds(0, hb - 1)], sem_b.at[2, s]),
            copy(k_hbm.at[hl], kb.at[s, hb - 1], sem_b.at[3, s]),
            copy(v_hbm.at[pl.ds(h0, hb)], vb.at[s], sem_b.at[4, s]),
        ]

    def b_o(i, s, j):
        return copy(ob.at[s, j], o_hbm.at[n_one + i * hb + j], sem_o.at[s, j])

    def run_blocks(zero):
        def body(it, carry):
            cur = it & 1
            nxt = 1 - cur
            loads = b_loads(jnp.minimum(it + 1, n_blk - 1), nxt)
            late_store = b_o(jnp.maximum(it - 1, 0), nxt, hb - 1)
            for c in loads:
                c.start()
            late_store.start()

            def slot(j):
                return ((n_one + j) & 1) + zero

            def prep_next(j, i):
                n1 = jnp.minimum(n_one + it * hb + j + 1, N - 1)
                prep(qb, kb, (cur, j), slot(j + 1), temp(n1) * _LOG2E, i)

            def after_head(j):
                if j < hb - 1:
                    b_o(it, cur, j).start()

            attend_bounded(_CFG_MAIN, hb, slot, vb, ob, lambda j: (cur, j),
                           prep_next, after_head)
            late_store.wait()
            for j in range(hb - 1):
                b_o(it, cur, j).wait()
            for c in loads:
                c.wait()
            return carry

        lax.fori_loop(0, n_blk, body, 0)
        last = b_o(n_blk - 1, (n_blk - 1) % 2, hb - 1)
        last.start()
        return last

    load_t = copy(t_hbm, t_ref, sem_t)
    load_t.start()
    first = [a_q(0, 0), a_k(0, 0)]
    second = [a_v(0, 0), a_q(min(1, N - 1), 1), a_k(min(1, N - 1), 1)]
    for c in first + second:
        c.start()
    oa[1] = jnp.zeros(oa.shape[1:], oa.dtype)
    load_t.wait()
    safe = None
    for i in range(H):
        ti = t_ref[i].astype(_F32)
        temp_ref[i] = ti
        ok = jnp.abs(ti) <= _T_SAFE
        safe = ok if safe is None else jnp.logical_and(safe, ok)
    for c in first:
        c.wait()
    scale0 = jnp.where(safe, temp_ref[0] * _LOG2E, 1.0)
    for i in range(npre):
        prep(qa, ka, (0,), 0, scale0, i)
    for c in second:
        c.wait()

    @pl.when(safe)
    def _bounded():
        if n_blk:
            for c in b_loads(0, 0):
                c.start()
            ob[1, hb - 1] = jnp.zeros(ob.shape[2:], ob.dtype)

        def attend(n, n1, cur, nxt):
            scale = temp(n1) * _LOG2E
            attend_bounded(_CFG_ONE, 1, lambda j: cur, va, oa, lambda j: (cur,),
                           lambda j, i: prep(qa, ka, (nxt,), nxt, scale, i),
                           lambda j: None)

        pending = [run_one_by_one(n_one, attend)]
        if n_blk:
            for c in b_loads(0, 0):
                c.wait()
            zero = (temp_ref[0] > 2 * _T_SAFE).astype(jnp.int32)
            pending.append(run_blocks(zero))
        for c in pending:
            c.wait()

    @pl.when(jnp.logical_not(safe))
    def _general():
        def attend(n, n1, cur, nxt):
            for i in range(npre):
                prep(qa, ka, (nxt,), nxt, 1.0, i)
            attend_general(n, cur)

        run_one_by_one(N, attend).wait()


@jax.jit
def pallas_standalone__qk_norm__prompt_kernel(
    q: jax.Array,
    k: jax.Array,
    v: jax.Array,
    t: jax.Array,
):
    B, H, S, D = q.shape
    N = B * H
    qt, kt, vt = (jnp.swapaxes(x, 2, 3).reshape(N, D, S) for x in (q, k, v))
    hbm = pl.BlockSpec(memory_space=pl.ANY)
    one = pltpu.VMEM((2, D, S), q.dtype)
    blk = pltpu.VMEM((2, _HB, D, S), q.dtype)
    o = pl.pallas_call(
        _kernel,
        in_specs=[hbm, hbm, hbm, hbm],
        out_specs=hbm,
        out_shape=jax.ShapeDtypeStruct((N, D, S), q.dtype),
        scratch_shapes=[
            one, one, one, one,
            blk, blk, blk, blk,
            pltpu.VMEM((3, S, D), _BF16),
            pltpu.VMEM((3, D, S), _BF16),
            pltpu.SMEM((H,), t.dtype),
            pltpu.SMEM((H,), _F32),
            pltpu.SemaphoreType.DMA((4, 2)),
            pltpu.SemaphoreType.DMA((5, 2)),
            pltpu.SemaphoreType.DMA((2, _HB)),
            pltpu.SemaphoreType.DMA,
        ],
        compiler_params=pltpu.CompilerParams(vmem_limit_bytes=48 * 1024 * 1024),
        name="qk_norm_attention",
    )(t, qt, kt, vt)
    return jnp.swapaxes(o.reshape(B, H, D, S), 2, 3)
```

```python
import jax
import jax.numpy as jnp
from jax import lax
import jax.experimental.pallas as pl
import jax.experimental.pallas.tpu as pltpu

_LOG2E = 1.4426950408889634
_EPS = 1e-6
_T_SAFE = 8.0
_F32 = jnp.float32
_BF16 = jnp.bfloat16

_HB = 4
_PC = 512
_SQ = 128
_CFG_ONE = (256, 512, 2, 0, 8)
_CFG_MAIN = (1024, 128, 1, 2, 4)


def _unit(x):
    x = x.astype(_F32)
    return x / (jnp.sqrt(jnp.sum(x * x, axis=0, keepdims=True)) + _EPS)


def _kernel(t_hbm, q_hbm, k_hbm, v_hbm, o_hbm,
            qa, ka, va, oa, rb, ob, ks_ref, qs_ref, t_ref, temp_ref,
            sem_a, sem_b, sem_o, sem_t):
    N, D, S = q_hbm.shape
    H = t_ref.shape[0]
    hb = _HB
    npre = S // _PC
    n_one = (N % hb or hb) if N >= 2 * hb else N
    n_blk = (N - n_one) // hb
    copy = pltpu.make_async_copy
    every = slice(None)

    def temp(n):
        return temp_ref[n & (H - 1) if H & (H - 1) == 0 else lax.rem(n, H)]

    def prep(qsrc, qidx, ksrc, kidx, slot, scale, i):
        sl = slice(i * _PC, (i + 1) * _PC)
        qs_ref[slot, :, sl] = (_unit(qsrc[qidx + (every, sl)]) * scale).astype(_BF16)
        ks_ref[slot, sl, :] = _unit(ksrc[kidx + (every, sl)]).T.astype(_BF16)

    def attend_bounded(cfg, nheads, slot, vsrc, vidx, odst, idx, prep_next, after_head):
        bq, bk, la, pstart, pevery = cfg
        nq, nk = S // bq, S // bk
        assert S % bq == 0 and S % bk == 0
        assert nq * nk > pevery * (pstart + npre - 1)
        steps = [(j, qi, ki) for j in range(nheads)
                 for qi in range(nq) for ki in range(nk)]

        def sdot(m):
            j, qi, ki = steps[m]
            return jnp.dot(ks_ref[slot(j), ki * bk:(ki + 1) * bk, :],
                           qs_ref[slot(j), :, qi * bq:(qi + 1) * bq],
                           preferred_element_type=_F32)

        pend = [sdot(m) for m in range(la)]
        issued = la
        acc = l = None
        for m, (j, qi, ki) in enumerate(steps):
            r = m % (nq * nk)
            ahead = la if m + la + 2 < len(steps) else la + 2
            while issued < min(len(steps), m + 1 + ahead):
                pend.append(sdot(issued))
                issued += 1
            if r % pevery == 0 and pstart <= r // pevery < pstart + npre:
                prep_next(j, r // pevery - pstart)
            p = jnp.exp2(pend.pop(0))
            ls = jnp.sum(p.reshape(bk // 8, 8, bq), axis=0)
            l = ls if ki == 0 else l + ls
            vt = vsrc[vidx(j) + (every, slice(ki * bk, (ki + 1) * bk))]
            pv = jnp.dot(vt, p.astype(_BF16), preferred_element_type=_F32)
            acc = pv if ki == 0 else acc + pv
            if ki == nk - 1:
                lsum = jnp.sum(l, axis=0, keepdims=True)
                odst[idx(j) + (every, slice(qi * bq, (qi + 1) * bq))] = (
                    acc / lsum).astype(odst.dtype)
                if qi == nq - 1:
                    after_head(j)

    def attend_general(n, cur):
        th = temp(n)

        def qblock(i, carry):
            col = pl.ds(pl.multiple_of(i * _SQ, _SQ), _SQ)
            s = jnp.dot(ks_ref[cur], qs_ref[cur, :, col],
                        preferred_element_type=_F32) * th
            p = jnp.exp(s - jnp.max(s, axis=0, keepdims=True))
            w = p / jnp.sum(p, axis=0, keepdims=True)
            o = jnp.dot(va[cur], w.astype(_BF16), preferred_element_type=_F32)
            oa[cur, :, col] = o.astype(oa.dtype)
            return carry

        lax.fori_loop(0, S // _SQ, qblock, 0)

    def a_q(n, s):
        return copy(q_hbm.at[n], qa.at[s], sem_a.at[0, s])

    def a_k(n, s):
        return copy(k_hbm.at[n], ka.at[s], sem_a.at[1, s])

    def a_v(n, s):
        return copy(v_hbm.at[n], va.at[s], sem_a.at[2, s])

    def a_o(n, s):
        return copy(oa.at[s], o_hbm.at[n], sem_a.at[3, s])

    def run_one_by_one(count, attend):
        top = min(count, N - 1)

        def body(n, carry):
            cur = n & 1
            nxt = 1 - cur
            n1 = jnp.minimum(n + 1, N - 1)
            n2 = jnp.minimum(n + 2, top)
            nv = jnp.minimum(n + 1, count - 1)
            nprev = jnp.maximum(n - 1, 0)
            loads = [a_q(n2, cur), a_k(n2, cur), a_v(nv, nxt)]
            store = a_o(nprev, nxt)
            for c in loads:
                c.start()
            store.start()
            attend(n, n1, cur, nxt)
            store.wait()
            for c in loads:
                c.wait()
            return carry

        lax.fori_loop(0, count, body, 0)
        last = a_o(count - 1, (count - 1) % 2)
        last.start()
        return last

    def b_loads(i, s):
        h0 = n_one + i * hb
        hl = jnp.minimum(h0 + hb, N - 1)
        sem = sem_b.at[s]
        return [
            copy(q_hbm.at[pl.ds(h0 + 1, hb - 1)], rb.at[s, 0, pl.ds(0, hb - 1)], sem),
            copy(q_hbm.at[hl], rb.at[s, 0, hb - 1], sem),
            copy(k_hbm.at[pl.ds(h0 + 1, hb - 1)], rb.at[s, 1, pl.ds(0, hb - 1)], sem),
            copy(k_hbm.at[hl], rb.at[s, 1, hb - 1], sem),
            copy(v_hbm.at[pl.ds(h0, hb)], rb.at[s, 2], sem),
        ]

    def b_loads_done(s):
        copy(rb.at[s], rb.at[s], sem_b.at[s]).wait()

    def b_o_early(i, s):
        return copy(ob.at[s, pl.ds(0, hb - 1)],
                    o_hbm.at[pl.ds(n_one + i * hb, hb - 1)], sem_o.at[s, 0])

    def b_o_late(i, s):
        return copy(ob.at[s, hb - 1], o_hbm.at[n_one + i * hb + hb - 1], sem_o.at[s, 1])

    def run_blocks(zero):
        def body(it, carry):
            cur = it & 1
            nxt = 1 - cur
            loads = b_loads(jnp.minimum(it + 1, n_blk - 1), nxt)
            late_store = b_o_late(jnp.maximum(it - 1, 0), nxt)
            for c in loads:
                c.start()
            late_store.start()

            def slot(j):
                return ((n_one + j) & 1) + zero

            def prep_next(j, i):
                n1 = jnp.minimum(n_one + it * hb + j + 1, N - 1)
                prep(rb, (cur, 0, j), rb, (cur, 1, j), slot(j + 1),
                     temp(n1) * _LOG2E, i)

            def after_head(j):
                if j == hb - 2:
                    b_o_early(it, cur).start()

            attend_bounded(_CFG_MAIN, hb, slot, rb, lambda j: (cur, 2, j),
                           ob, lambda j: (cur, j), prep_next, after_head)
            late_store.wait()
            b_o_early(it, cur).wait()
            b_loads_done(nxt)
            return carry

        lax.fori_loop(0, n_blk, body, 0)
        last = b_o_late(n_blk - 1, (n_blk - 1) % 2)
        last.start()
        return last

    load_t = copy(t_hbm, t_ref, sem_t)
    load_t.start()
    first = [a_q(0, 0), a_k(0, 0)]
    second = [a_v(0, 0), a_q(min(1, N - 1), 1), a_k(min(1, N - 1), 1)]
    for c in first + second:
        c.start()
    oa[1] = jnp.zeros(oa.shape[1:], oa.dtype)
    load_t.wait()
    safe = None
    for i in range(H):
        ti = t_ref[i].astype(_F32)
        temp_ref[i] = ti
        ok = jnp.abs(ti) <= _T_SAFE
        safe = ok if safe is None else jnp.logical_and(safe, ok)
    for c in first:
        c.wait()
    scale0 = jnp.where(safe, temp_ref[0] * _LOG2E, 1.0)
    for i in range(npre):
        prep(qa, (0,), ka, (0,), 0, scale0, i)
    for c in second:
        c.wait()

    @pl.when(safe)
    def _bounded():
        if n_blk:
            for c in b_loads(0, 0):
                c.start()
            ob[1, hb - 1] = jnp.zeros(ob.shape[2:], ob.dtype)

        def attend(n, n1, cur, nxt):
            scale = temp(n1) * _LOG2E
            attend_bounded(_CFG_ONE, 1, lambda j: cur, va, lambda j: (cur,),
                           oa, lambda j: (cur,),
                           lambda j, i: prep(qa, (nxt,), ka, (nxt,), nxt, scale, i),
                           lambda j: None)

        pending = [run_one_by_one(n_one, attend)]
        if n_blk:
            b_loads_done(0)
            zero = (temp_ref[0] > 2 * _T_SAFE).astype(jnp.int32)
            pending.append(run_blocks(zero))
        for c in pending:
            c.wait()

    @pl.when(jnp.logical_not(safe))
    def _general():
        def attend(n, n1, cur, nxt):
            for i in range(npre):
                prep(qa, (nxt,), ka, (nxt,), nxt, 1.0, i)
            attend_general(n, cur)

        run_one_by_one(N, attend).wait()


@jax.jit
def pallas_standalone__qk_norm__prompt_kernel(
    q: jax.Array,
    k: jax.Array,
    v: jax.Array,
    t: jax.Array,
):
    B, H, S, D = q.shape
    N = B * H
    qt, kt, vt = (jnp.swapaxes(x, 2, 3).reshape(N, D, S) for x in (q, k, v))
    hbm = pl.BlockSpec(memory_space=pl.ANY)
    one = pltpu.VMEM((2, D, S), q.dtype)
    o = pl.pallas_call(
        _kernel,
        in_specs=[hbm, hbm, hbm, hbm],
        out_specs=hbm,
        out_shape=jax.ShapeDtypeStruct((N, D, S), q.dtype),
        scratch_shapes=[
            one, one, one, one,
            pltpu.VMEM((2, 3, _HB, D, S), q.dtype),
            pltpu.VMEM((2, _HB, D, S), q.dtype),
            pltpu.VMEM((3, S, D), _BF16),
            pltpu.VMEM((3, D, S), _BF16),
            pltpu.SMEM((H,), t.dtype),
            pltpu.SMEM((H,), _F32),
            pltpu.SemaphoreType.DMA((4, 2)),
            pltpu.SemaphoreType.DMA((2,)),
            pltpu.SemaphoreType.DMA((2, 2)),
            pltpu.SemaphoreType.DMA,
        ],
        compiler_params=pltpu.CompilerParams(vmem_limit_bytes=48 * 1024 * 1024),
        name="qk_norm_attention",
    )(t, qt, kt, vt)
    return jnp.swapaxes(o.reshape(B, H, D, S), 2, 3)
```
